```python
import os as _os
_os.environ.setdefault("JAX_PLATFORMS", "cpu")
import jax
import jax.numpy as jnp

def _softmax(x, axis=-1):
    return jax.nn.softmax(x, axis=axis)
def _gelu(x):
    return jax.nn.gelu(x, approximate=True)
def _silu(x):
    return jax.nn.silu(x)
def _sigmoid(x):
    return jax.nn.sigmoid(x)
def _layernorm(x, axis=-1, eps=1e-5):
    m = jnp.mean(x, axis=axis, keepdims=True)
    v = jnp.var(x, axis=axis, keepdims=True)
    return (x - m) / jnp.sqrt(v + eps)
def _scatter_add(tgt, idx, src, axis=0):
    return tgt.at[idx].add(src)
def _segment_sum(src, seg, n):
    return jax.ops.segment_sum(src, seg, n)
class _Rng:
    def __init__(self, key):
        self._k = key
    def _next(self):
        self._k, sub = jax.random.split(self._k)
        return sub
    def normal(self, shape):
        return jax.random.normal(self._next(), shape, dtype=jnp.bfloat16)
    def randint(self, lo, hi, shape):
        return jax.random.randint(self._next(), shape, lo, hi, dtype=jnp.int32)
    def uniform(self, shape, lo=0.0, hi=1.0):
        return jax.random.uniform(self._next(), shape, jnp.bfloat16, lo, hi)
    def permutation(self, n):
        return jax.random.permutation(self._next(), n)


kernel_name = 'recurrent_scan__spectral_gfnet__swiglu_ffn__prompt'

def setup_inputs():
    _rng = _Rng(jax.random.key(int.from_bytes(__import__("os").urandom(4), "little")))
    _w = (lambda a: (lambda t: t.astype(jnp.bfloat16) if jnp.issubdtype(t.dtype, jnp.floating) else t)(jnp.asarray(a)))
    def _A_setup():
        B, S, D = 1, 2048, 640
        Df = D // 2 + 1
        return {
            "x": _w((lambda *s: _rng.normal(s) * 0.05)(B, S, D)),
            "w_r": _w((lambda *s: _rng.normal(s) * 0.05)(S, Df) * 0.02),
            "w_i": _w((lambda *s: _rng.normal(s) * 0.05)(S, Df) * 0.02),
        }
    _A_in = _A_setup()

    def _B_setup():
        B, S, D, F = 1, 2048, 640, 1536
        return {
            "x": _w((lambda *s: _rng.normal(s) * 0.05)(B, S, D)),
            "w_gate": _w((lambda *s: _rng.normal(s) * 0.05)(D, F)),
            "w_up": _w((lambda *s: _rng.normal(s) * 0.05)(D, F)),
            "w_down": _w((lambda *s: _rng.normal(s) * 0.05)(F, D)),
        }
    _B_in = _B_setup()

    return {
        "A_x": _A_in["x"],
        "A_w_r": _A_in["w_r"],
        "A_w_i": _A_in["w_i"],
        "B_x": _B_in["x"],
        "B_w_gate": _B_in["w_gate"],
        "B_w_up": _B_in["w_up"],
        "B_w_down": _B_in["w_down"],
    }

def reference(A_x, A_w_r, A_w_i, B_x, B_w_gate, B_w_up, B_w_down):
    def _A_ref(x, w_r, w_i):
        B, S, D = x.shape
        X = (lambda x, axes=(-2,-1): jnp.fft.rfft2(x.astype(jnp.float32), axes=axes))(x, axes=(-2, -1))
        W = w_r + 1j * w_i
        X = X * W
        y = (lambda x, s, axes=(-2,-1): jnp.fft.irfft2(x, s=s, axes=axes).astype(jnp.bfloat16))(X, (S, D), axes=(-2, -1))
        return y

    def _B_ref(x, w_gate, w_up, w_down):
        g = _silu(x @ w_gate)
        u = x @ w_up
        return (g * u) @ w_down

    x = A_x
    xn = _layernorm(x, axis=-1)
    s = _A_ref(xn, A_w_r, A_w_i)
    g = _silu(_B_ref(xn, B_w_gate, B_w_up, B_w_down))
    return x + s * g
```

```python
import numpy as np
import jax
import jax.numpy as jnp
from jax import lax
import jax.experimental.pallas as pl
import jax.experimental.pallas.tpu as pltpu

S, D, F = 2048, 640, 1536
DF = D // 2 + 1
N1, N2 = 32, 64
L = 128
RB = 256
MB = 512
MS = 128
WP = N1 + 1
QD, QF = 16, 16
CUTS = (0, 3, 5, 9, 12, 14, 19, 25)
SUB = 32
FC = 256
SH = MB // 2
KH = 256
BF = jnp.bfloat16
F32 = jnp.float32


def _constants():
    H = L // 2

    def block(l, nb, sg):
        th = 2 * np.pi * ((np.arange(nb)[:, None] * l[None, :]) % D) / D
        co, si = np.cos(th), np.sin(th)
        wt = np.where((l == 0) | (l == D // 2), 1.0, 2.0) / (S * D)
        return np.block([[co, -si], [-_S1 * sg * si, -_S1 * sg * co]]), np.concatenate([wt, wt])

    j = 10 * np.arange(H // 2)
    m, wt = block(np.concatenate([j, j + 5, [D // 2]]), L, 1.0)
    keep = np.concatenate([np.arange(H + 1), H + 2 + np.arange(H - 1)])
    tiles = [(m[:L, keep], wt[keep])]
    for c in (1, 2):
        for cc in (c, c + 5):
            m, wt = block(np.concatenate([cc + j, 10 - cc + j]), H, np.repeat([1.0, -1.0], H // 2))
            tiles.append((m if cc == c else np.roll(m, H, 1), wt))
    fd = np.concatenate([m for m, _ in tiles], 1)
    fi = np.concatenate([(m * wt).T for m, wt in tiles], 1)
    k = (np.arange(N1)[:, None, None] + N1 * np.arange(N2)[None, :, None])
    ph = 2 * np.pi * ((k * np.arange(N2)[None, None, :]) % S) / S
    co, si = np.cos(ph), np.sin(ph)
    g = np.concatenate([np.concatenate([co, si], 2), np.concatenate([-si, co], 2)], 1)
    gi = np.transpose(g, (0, 2, 1))

    def cast(a):
        h = np.asarray(a, np.float32).astype(BF).view(np.uint16).astype(np.uint32)
        return h[..., 0::2, :] | (h[..., 1::2, :] << 16)

    return cast(fd), cast(fi), cast(g), cast(gi)


_C1, _C2 = float(np.cos(2 * np.pi / 5)), float(np.cos(4 * np.pi / 5))
_S1, _S2 = float(np.sin(2 * np.pi / 5)), float(np.sin(4 * np.pi / 5))


def _cmulc(z, num, den, sign):
    re, im = z
    num %= den
    if num == 0:
        return z
    if 4 * num == den:
        return (-im, re) if sign > 0 else (im, -re)
    if 2 * num == den:
        return (-re, -im)
    if 4 * num == 3 * den:
        return (im, -re) if sign > 0 else (-im, re)
    c = float(np.cos(2 * np.pi * num / den))
    s = float(sign * np.sin(2 * np.pi * num / den))
    if (8 * num) % den == 0:
        a = abs(c)
        p, m = re + im, re - im
        if c > 0 and s > 0:
            return (m * a, p * a)
        if c > 0 and s < 0:
            return (p * a, m * (-a))
        if c < 0 and s > 0:
            return (p * (-a), m * a)
        return (m * (-a), p * (-a))
    return (re * c - im * s, re * s + im * c)


def _fft(zs, sign):
    n = len(zs)
    if n == 1:
        return zs
    ev, od = _fft(zs[0::2], sign), _fft(zs[1::2], sign)
    out = [None] * n
    for k in range(n // 2):
        e = ev[k]
        if 4 * k == n:
            o = od[k]
            if sign > 0:
                out[k], out[k + n // 2] = (e[0] - o[1], e[1] + o[0]), (e[0] + o[1], e[1] - o[0])
            else:
                out[k], out[k + n // 2] = (e[0] + o[1], e[1] - o[0]), (e[0] - o[1], e[1] + o[0])
        else:
            o = _cmulc(od[k], k, n, sign)
            out[k], out[k + n // 2] = (e[0] + o[0], e[1] + o[1]), (e[0] - o[0], e[1] - o[1])
    return out


def _silu(v):
    hv = 0.5 * v
    return hv * jnp.tanh(hv) + hv


def _interleave(*gens):
    done = [0] * len(gens)
    total = max(n for _, n in gens)
    for t in range(1, total + 1):
        for i, (g, n) in enumerate(gens):
            while done[i] * total < t * n:
                next(g)
                done[i] += 1
    for g, _ in gens:
        assert next(g, _END) is _END


_END = object()


class _Packed:
    def __init__(self, ref):
        self.ref = ref

    @staticmethod
    def _idx(idx):
        *lead, rows, cols = idx
        lo, n = (rows.start, rows.size) if isinstance(rows, pl.Slice) else (rows.start, rows.stop - rows.start)
        return (*lead, pl.ds(lo // 2, n // 2), cols)

    def __getitem__(self, idx):
        return pltpu.bitcast(self.ref[self._idx(idx)], BF)

    def __setitem__(self, idx, val):
        self.ref[self._idx(idx)] = pltpu.bitcast(val, jnp.uint32)


def _kernel(x_hbm, wr_hbm, wi_hbm, wg_hbm, wu_hbm, wd_hbm, fd_hbm, fi_hbm, g_hbm, gi_hbm,
            o_hbm,
            x_v, wr_v, wi_v, wg_v, wu_v, wd_v, fd_v, fi_v, g_v, gi_v,
            xn_v, yb_v, y_v, b_v, t_v, wn_v, wp_v, gate_v, h_v, sw_v, sx_v, sd_v, sh_v, act_v, o_v, sem_x, sem_f, sem_w, sem_o, sem_b):
    nb, nf = S // RB, F // FC
    U32 = jnp.uint32
    blk = lambda i: pl.ds(i * RB, RB)
    x_cp = lambda i: pltpu.make_async_copy(x_hbm.at[blk(i)], x_v.at[blk(i)], sem_x.at[i])
    o_cp = lambda r, n: pltpu.make_async_copy(o_v.at[pl.ds(r, n)], o_hbm.at[pl.ds(r, n)], sem_o.at[r // MS])
    end_cp = [pltpu.make_async_copy(o_v.at[S - MS:S, cs], o_hbm.at[S - MS:S, cs], sem_o.at[1 + i])
              for i, cs in enumerate((slice(0, D - L), slice(D - L, D)))]
    cut = [0, FC // 2] + [f * FC for f in range(1, nf + 1)]
    f_cp = [[pltpu.make_async_copy(a.at[:, lo:hi], b.at[:, lo:hi], sem_f.at[2 * f + j])
             for j, (a, b) in enumerate(((wg_hbm, wg_v), (wu_hbm, wu_v)))]
            for f, (lo, hi) in enumerate(zip(cut, cut[1:]))]
    f0a_cp = f_cp.pop(0)
    pairs = [(fd_hbm, fd_v), (wd_hbm, wd_v), (g_hbm, g_v), (gi_hbm, gi_v),
             (fi_hbm, fi_v), (wr_hbm, wr_v), (wi_hbm, wi_v)]
    fd_cp, wd_cp, g_cp, gi_cp, fi_cp, *w_cp = [
        pltpu.make_async_copy(a, b, sem_w.at[i]) for i, (a, b) in enumerate(pairs)]
    fd_v, fi_v, g_v, gi_v, xn_v, yb_v, h_v, sw_v, sx_v, sd_v, sh_v = map(
        _Packed, (fd_v, fi_v, g_v, gi_v, xn_v, yb_v, h_v, sw_v, sx_v, sd_v, sh_v))
    queue = [[x_cp(0)], f0a_cp, f_cp[0], [x_cp(1)], f_cp[1], f_cp[2], [x_cp(2), x_cp(3)], f_cp[3], f_cp[4],
             [x_cp(4), x_cp(5)], f_cp[5], [fd_cp, x_cp(6), x_cp(7)], w_cp, [wd_cp], [g_cp], [gi_cp],
             [fi_cp]]

    def start(n):
        for grp in queue[:n]:
            for c in grp:
                c.start()
        del queue[:n]

    def wait(*cs):
        for c in cs:
            c.wait()

    lane = lambda n: lax.broadcasted_iota(jnp.int32, (n, L), 1)
    swap = lambda v: pltpu.roll(v, L // 2, 1)

    def halves(n, c):
        low = lane(n) < L // 2
        co, si = float(np.cos(2 * np.pi * c / 10)), float(np.sin(2 * np.pi * c / 10))
        return low, co, jnp.where(low, -_S1 * si, si / _S1)

    def ln(*blocks, serial=True, fuse=True):
        zero = None
        for q in range(blocks[0] * RB // SUB, (blocks[-1] + 1) * RB // SUB):
            rows = pl.ds(q * SUB, SUB)
            x = x_v[rows, :].astype(F32)
            tot = sum(x[:, a * L:(a + 1) * L] for a in range(1, D // L)) + x[:, :L]
            if zero is not None:
                tot = tot + zero
            xc = x - jnp.sum(tot, axis=-1, keepdims=True) * (1.0 / D)
            var = jnp.mean(xc * xc, axis=-1, keepdims=True)
            rstd = lax.rsqrt(var + 1e-5)
            if serial:
                zero = pltpu.bitcast(pltpu.bitcast(jnp.broadcast_to(rstd, (SUB, L)), U32) >> 31, F32)
            xn = xc * rstd
            xn_v[rows, :] = xn.astype(BF)
            if fuse:
                radix10(rows, xn)
            yield

    def butterflies(i):
        for q in range(RB // SUB):
            rows = pl.ds(i * RB + q * SUB, SUB)
            radix10(rows, xn_v[rows, :].astype(F32))
            yield

    def radix10(rows, xn):
        x0, x1, x2, x3, x4 = [xn[:, a * L:(a + 1) * L] for a in range(5)]
        t1, t2, t3, t4 = x1 + x4, x2 + x3, x1 - x4, x2 - x3
        t5 = t1 + t2
        m1, m2 = x0 - 0.25 * t5, (0.5 * (_C1 - _C2)) * (t1 - t2)
        ys = [x0 + t5]
        for c, er, ei in ((1, m1 + m2, t3 + (_S2 / _S1) * t4), (2, m1 - m2, (_S2 / _S1) * t3 - t4)):
            low, co, sv = halves(SUB, c)
            rr, ri = swap(er), swap(ei)
            lo = jnp.where(low, er, ri)
            hi = co * jnp.where(low, rr, ei) + sv * jnp.where(low, ri, er)
            ys += [lo + hi, lo - hi]
        for a, yv in enumerate(ys):
            yb_v[rows, a * L:(a + 1) * L] = yv.astype(BF)

    quarters = lambda q, e, n: [pl.ds(S // 4 * p + N2 * q + n * e, n) for p in range(4)]
    split = lambda re, im: [(re[QD * p:QD * p + QD], im[QD * p:QD * p + QD]) for p in range(4)]

    def dmat():
        for q in range(8):
            for e in range(N2 // QD):
                rs = quarters(q, e, QD)
                tile = lambda a: jnp.dot(jnp.concatenate([yb_v[r, a * L:(a + 1) * L] for r in rs], 0),
                                         fd_v[0:L, a * L:(a + 1) * L], preferred_element_type=F32)
                for c in range(3):
                    if c == 0:
                        re = tile(0)
                        im = jnp.where(lane(4 * QD) % (L // 2) == 0, 0.0, swap(re))
                    else:
                        low = lane(4 * QD) < L // 2
                        t1, t2 = tile(2 * c - 1), tile(2 * c)
                        re, im = jnp.where(low, t1, t2), swap(jnp.where(low, t2, t1))
                    for u, z in enumerate(_fft(split(re, im), -1)):
                        z = _cmulc(z, q * u, N1, -1)
                        y_v[c, 0, rs[u], :] = z[0]
                        y_v[c, 1, rs[u], :] = z[1]
                    yield

    def wcomb(k, f):
        ref, c1, c2 = (wg_v, wu_v)[k], slice(f * FC, (f + 1) * FC), slice((f + 1) * FC, (f + 2) * FC)
        for r in range(0, KH, 16):
            b11, b21, b12, b22 = (ref[o + r:o + r + 16, c].astype(F32) for c in (c1, c2) for o in (0, KH))
            for i, v in enumerate((b11 + b22, b12 - b22, b21 - b11, b11 + b12, b21 + b22)):
                sw_v[i, r:r + 16, (f + k) * FC:(f + k + 1) * FC] = v.astype(BF)
            yield

    def xcomb(m):
        for top in range(m * MB, (m + 1) * MB, 2 * SH):
            for r in range(0, SH, 16):
                a11, a12, a21, a22 = (xn_v[pl.ds(top + o + r, 16), c:c + KH].astype(F32)
                                      for o in (0, SH) for c in (0, KH))
                for i, v in enumerate((a11 + a22, a21 + a22, a11 + a12, a21 - a11, a12 - a22)):
                    sx_v[i, pl.ds((top - MB) // 2 + r, 16), 0:KH] = v.astype(BF)
                yield

    def matmul7(k, top, f, emit):
        ref, c1, c2 = (wg_v, wu_v)[k], slice(f * FC, (f + 1) * FC), slice((f + 1) * FC, (f + 2) * FC)
        mm = lambda a, b: jnp.dot(a, b, preferred_element_type=F32)
        rt, rb = pl.ds(top, SH), pl.ds(top + SH, SH)
        sx = lambda i: sx_v[i, pl.ds((top - MB) // 2, SH), 0:KH]
        sw = lambda i: sw_v[i, 0:KH, (f + k) * FC:(f + k + 1) * FC]
        m2 = mm(sx(1), ref[0:KH, c1])
        yield
        m4 = mm(xn_v[rb, KH:2 * KH], sw(2))
        yield
        emit(1, 0, m2 + m4 + mm(xn_v[rb, 2 * KH:D], ref[2 * KH:D, c1]))
        yield
        m3 = mm(xn_v[rt, 0:KH], sw(1))
        yield
        m1 = mm(sx(0), sw(0))
        yield
        m6 = mm(jnp.concatenate([sx(3), xn_v[rb, 2 * KH:D]], 1), jnp.concatenate([sw(3), ref[2 * KH:D, c2]], 0))
        emit(1, 1, (m1 - m2) + (m3 + m6))
        yield
        m5 = mm(sx(2), ref[KH:2 * KH, c2])
        yield
        emit(0, 1, m3 + m5 + mm(xn_v[rt, 2 * KH:D], ref[2 * KH:D, c2]))
        yield
        m7 = mm(jnp.concatenate([sx(4), xn_v[rt, 2 * KH:D]], 1), jnp.concatenate([sw(4), ref[2 * KH:D, c1]], 0))
        emit(0, 0, (m1 + m4) + (m7 - m5))
        yield

    def gate_up7(top, j):
        def gate(i, c, v):
            act_v[i, c] = _silu(v)

        def up(i, c, v):
            cs = slice((j - 1 + c) * FC, (j + c) * FC)
            h_v[pl.ds((top + i * SH) % (2 * MB), SH), cs] = (act_v[i, c] * v).astype(BF)

        return matmul7(j % 2, top, j - j % 2, up if j % 2 else gate)

    def dcomb():
        for p in range(nf // 2):
            for r in range(0, FC, 16):
                b11, b21, b12, b22 = (wd_v[(2 * p + o) * FC + r:(2 * p + o) * FC + r + 16, c:c + FC].astype(F32)
                                      for c in (0, FC) for o in (0, 1))
                for i, v in enumerate((b11 + b22, b12 - b22, b21 - b11, b11 + b12, b21 + b22)):
                    sd_v[i, p * FC + r:p * FC + r + 16, 0:FC] = v.astype(BF)
                yield

    def hcomb(m, p):
        for r in range(0, SH, 16):
            a11, a12, a21, a22 = (h_v[pl.ds(m % 2 * MB + o + r, 16), (2 * p + c) * FC:(2 * p + c + 1) * FC].astype(F32)
                                  for o in (0, SH) for c in (0, 1))
            for i, v in enumerate((a11 + a22, a21 + a22, a11 + a12, a21 - a11, a12 - a22)):
                sh_v[m % 2, i, r:r + 16, p * FC:(p + 1) * FC] = v.astype(BF)
            yield

    def down7(top):
        slot = top // MB % 2
        ch = lambda p, c: slice((2 * p + c) * FC, (2 * p + c + 1) * FC)
        sh = lambda i: (lambda p: sh_v[slot, i, 0:SH, p * FC:(p + 1) * FC])
        sd = lambda i: (lambda p: sd_v[i, p * FC:(p + 1) * FC, 0:FC])
        res = []

        def prod(a, b):
            acc = None
            for p in range(nf // 2):
                d = jnp.dot(a(p), b(p), preferred_element_type=F32)
                acc = d if acc is None else acc + d
                if p == nf // 2 - 1:
                    res.append(acc)
                else:
                    yield

        def emit(i, c, v):
            gate_v[pl.ds(top + i * SH, SH), c * FC:(c + 1) * FC] = _silu(v)

        yield from prod(sh(1), lambda p: wd_v[ch(p, 0), 0:FC])
        yield
        yield from prod(lambda p: h_v[pl.ds(slot * MB + SH, SH), ch(p, 1)], sd(2))
        emit(1, 0, res[0] + res[1])
        yield
        yield from prod(lambda p: h_v[pl.ds(slot * MB, SH), ch(p, 0)], sd(1))
        yield
        yield from prod(sh(0), sd(0))
        yield
        yield from prod(sh(3), sd(3))
        m2, m4, m3, m1, m6 = res
        emit(1, 1, (m1 - m2) + (m3 + m6))
        yield
        yield from prod(sh(2), lambda p: wd_v[ch(p, 1), FC:2 * FC])
        emit(0, 1, m3 + res[5])
        yield
        yield from prod(sh(4), sd(4))
        emit(0, 0, (m1 + m4) + (res[6] - res[5]))
        yield

    def mlp(items, ms, part=(0, FC)):
        for r0, rows, j in items:
            if j < 0:
                yield from down7(r0)
                continue
            if j < nf and r0 >= MB:
                for r in range(r0, r0 + rows, 2 * SH):
                    yield from gate_up7(r, j)
                continue
            for r in range(r0, r0 + rows, ms):
                hr = pl.ds(r % (2 * MB), ms)
                if j < nf:
                    cs = slice(j * FC + part[0], j * FC + part[1])
                    xb = xn_v[pl.ds(r, ms), :]
                    a = jnp.dot(xb, wg_v[0:D, cs], preferred_element_type=F32)
                    yield
                    u = jnp.dot(xb, wu_v[0:D, cs], preferred_element_type=F32)
                    h_v[hr, cs] = (_silu(a) * u).astype(BF)
                else:
                    cs = slice((j - nf) * L, (j - nf + 1) * L)
                    rs = pl.ds(r, ms)
                    gt = _silu(jnp.dot(h_v[hr, :], wd_v[0:F, cs], preferred_element_type=F32))
                    if r < S - MB:
                        gate_v[rs, cs] = gt
                    else:
                        o_v[rs, cs] = (x_v[rs, cs].astype(F32) + gate_v[rs, cs] * gt).astype(BF)
                        if r + ms == S and j >= nf + D // L - 2:
                            end_cp[j - nf - D // L + 2].start()
                        elif j == nf + D // L - 1:
                            o_cp(r, ms).start()
                yield

    def mlp_stream(items, ms, *part):
        steps = lambda r0, rows, j: (21 if j < 0 else rows // ms if j >= nf else 2 * rows // ms if r0 < MB else 9 * rows // (2 * SH))
        return mlp(items, ms, *part), sum(steps(*it) for it in items)

    def wprep():
        for i in range(S // L):
            cols = slice(i * L, (i + 1) * L)
            for j, ref in enumerate((wr_v, wi_v)):
                for r in range(0, DF - 1, 64):
                    wn_v[i % 2, j, r // 2:r // 2 + 32, :] = pltpu.bitcast(ref[r:r + 64, cols], U32)

            def sel(d):
                wr, wi = (wn_v[i % 2, j, pl.ds(d // 2, L // 4, stride=5), :] for j in range(2))
                return (wr & np.uint32(0xFFFF0000)) | (wi >> 16) if d % 2 else (wr << 16) | (wi & np.uint32(0xFFFF))

            nr, ni = (pltpu.bitcast(jnp.broadcast_to(ref[DF - 1:DF, cols].astype(F32), (8, L)), U32)
                      for ref in (wr_v, wi_v))
            nyq = jnp.where(lax.broadcasted_iota(jnp.int32, (8, L), 0) == 0, nr | (ni >> 16), np.uint32(0))
            for c, ds in enumerate(((0, 5), (1, 9, 6, 4), (2, 8, 7, 3))):
                rows = [sel(d) for d in ds] + ([] if c else [nyq, jnp.zeros((L // 2 - 8, L), U32)])
                t = jnp.concatenate(rows, 0).T
                for g in range(L // N1):
                    wp_v[c, pl.ds(WP * (L // N1 * i + g), N1), :] = t[N1 * g:N1 * (g + 1)]
                yield

    at = lambda s1, j: pl.ds(N2 * s1 + 8 * j, 8)

    def fwd(c):
        for j in range(N2 // 8):
            for u in range(4):
                zs = [(y_v[c, 0, at(8 * u + q, j), :], y_v[c, 1, at(8 * u + q, j), :]) for q in range(8)]
                for v, z in enumerate(_fft(zs, -1)):
                    t_v[c, u + 4 * v, at(0, j), :] = z[0]
                    t_v[c, u + 4 * v, at(1, j), :] = z[1]
                yield

    def filt(c):
        for k1 in range(N1):
            r = jnp.dot(g_v[k1, 0:L, :], t_v[c, k1].astype(BF), preferred_element_type=F32)
            word = wp_v[c, pl.ds(k1, N2, stride=WP), :]
            wr = pltpu.bitcast(word & np.uint32(0xFFFF0000), F32)
            wi = pltpu.bitcast(word << 16, F32)
            xr, xi = r[:N2], r[N2:]
            zz = jnp.concatenate([xr * wr - xi * wi, xr * wi + xi * wr], 0).astype(BF)
            b = jnp.dot(gi_v[k1, 0:L, :], zz, preferred_element_type=F32)
            b_v[c, 0, pl.ds(N2 * k1, N2), :] = b[:N2]
            b_v[c, 1, pl.ds(N2 * k1, N2), :] = b[N2:]
            if k1 % 2:
                yield

    def inv(c):
        for j in range(N2 // 8):
            for u in range(4):
                zs = [(b_v[c, 0, at(u + 4 * v, j), :], b_v[c, 1, at(u + 4 * v, j), :]) for v in range(8)]
                for q, z in enumerate(_fft(zs, 1)):
                    z = _cmulc(z, q * u, N1, 1)
                    y_v[c, 0, at(8 * u + q, j), :] = z[0]
                    y_v[c, 1, at(8 * u + q, j), :] = z[1]
                yield

    def finish():
        tile = lambda a, v: jnp.dot(v.astype(BF), fi_v[0:L, a * L:(a + 1) * L], preferred_element_type=F32)
        for q in range(8):
            for e in range(N2 // QF):
                rs = quarters(q, e, QF)

                def load(c):
                    zs = _fft([(y_v[c, 0, r, :], y_v[c, 1, r, :]) for r in rs], 1)
                    return jnp.concatenate([z[0] for z in zs], 0), swap(jnp.concatenate([z[1] for z in zs], 0))

                us = []
                for c in (1, 2):
                    low, co, _ = halves(4 * QF, c)
                    zr, zi = load(c)
                    v1, v2 = tile(2 * c - 1, jnp.where(low, zr, zi)), tile(2 * c, jnp.where(low, zi, zr))
                    yield
                    ad, df = v1 + v2, v1 - v2
                    si = float(np.sin(2 * np.pi * c / 10))
                    ds = swap(df)
                    us += [jnp.where(low, ad, co * ds + (si / _S1) * df),
                           jnp.where(low, swap(ad), co * df - (_S1 * si) * ds)]
                u0 = tile(0, jnp.where(lane(4 * QF) <= L // 2, *load(0)))
                yield
                u1r, u1i, u2r, u2i = us
                t5 = u1r + u2r
                m1, m2 = u0 - 0.25 * t5, (0.5 * (_C1 - _C2)) * (u1r - u2r)
                e1, e2 = m1 + m2, m1 - m2
                d1, d2 = u1i + (_S2 / _S1) * u2i, (_S2 / _S1) * u1i - u2i
                for a, sp in enumerate((u0 + t5, e1 + d1, e2 + d2, e2 - d2, e1 - d1)):
                    cs = slice(a * L, (a + 1) * L)
                    for p, r in enumerate(rs):
                        if p < 3:
                            o_v[r, cs] = (x_v[r, cs].astype(F32) + sp[QF * p:QF * p + QF] * gate_v[r, cs]).astype(BF)
                        else:
                            gate_v[r, cs] = sp[QF * p:QF * p + QF]
                yield

    def fence():
        pl.semaphore_signal(sem_b, 1)
        pl.semaphore_wait(sem_b, 1)

    def chain(*gens):
        for g in gens:
            yield from g

    nq, nd = RB // SUB, D // L
    each = lambda fn, ids: chain(*[fn(i) for i in ids])
    start(4)
    wp_v[...] = jnp.zeros(wp_v.shape, U32)
    wn_v[...] = jnp.zeros(wn_v.shape, U32)
    wait(x_cp(0))
    _interleave((ln(0, serial=False, fuse=False), nq))
    wait(*f0a_cp)
    start(1)
    _interleave(mlp_stream([(0, RB, 0)], RB, (0, FC // 2)))
    wait(*f_cp[0])
    start(2)
    _interleave(mlp_stream([(0, RB, 0)], RB, (FC // 2, FC)))
    first = lambda js: [(0, MB, j) for j in js]
    wait(x_cp(1))
    start(1)
    _interleave((ln(1, serial=False, fuse=False), nq))
    _interleave(mlp_stream([(RB, RB, 0)], MS))
    wait(*f_cp[1])
    start(2)
    _interleave(mlp_stream(first([1]), MS), (butterflies(0), nq), (wcomb(0, 0), 16))
    wait(*f_cp[2], x_cp(2), x_cp(3))
    start(3)
    _interleave(mlp_stream(first([2]), MS), (ln(2, fuse=False), nq), (ln(3, fuse=False), nq))
    wait(*f_cp[3], *f_cp[4])
    start(1)
    fence()
    _interleave(mlp_stream(first([3, 4]), MS), (each(butterflies, (1, 2, 3)), 3 * nq), (chain(wcomb(1, 0), xcomb(1)), 32))
    wait(*f_cp[5], fd_cp, *[x_cp(i) for i in range(4, nb)])
    gu = lambda m: [(m * MB, MB, j) for j in range(nf)]
    dn = lambda m: [(m * MB, MB, nf + nd - 1), (m * MB, MB, -1)]
    items = first([5]) + gu(1) + [dn(0)[0], dn(1)[0], dn(0)[1], dn(1)[1]] + gu(2) + dn(2) + gu(3)
    hsums = lambda m, ps: (chain(*[hcomb(m, p) for p in ps]), 16 * len(ps))
    extra = {9: hsums(1, range(3)), 15: hsums(2, [0]), 16: hsums(2, [1]), 17: hsums(2, [2])}

    def mix(a, na, b, nb_):
        for t in range(na):
            next(a)
            for _ in range(nb_ * (t + 1) // na - nb_ * t // na):
                next(b)
            yield

    def part(i, ms):
        gs = [mlp_stream([items[k]], ms) for k in range(CUTS[i], CUTS[i + 1])]
        gs = [(mix(g, n, *extra[k]) if k in extra else g, n) for k, (g, n) in enumerate(gs, CUTS[i])]
        return chain(*[g for g, _ in gs]), sum(n for _, n in gs)

    start(1)
    fence()
    _interleave(part(0, RB), (ln(4, 5), 2 * nq), (ln(6, 7), 2 * nq), (chain(wcomb(0, 2), wcomb(1, 2)), 32))
    wait(*w_cp)
    fence()
    start(len(queue))
    _interleave(part(1, RB), (wprep(), 48), (chain(wcomb(0, 4), wcomb(1, 4)), 32))
    wait(wd_cp)
    fence()
    _interleave(part(2, MS), (dmat(), 24 * N2 // QD), (dcomb(), 48), hsums(0, range(3)))
    fence()
    _interleave(part(3, MS), (each(fwd, range(3)), 96), (chain(xcomb(2), iter([None] * 8)), 24))
    wait(g_cp, gi_cp)
    _interleave(part(4, RB), (each(filt, range(3)), 48), (xcomb(3), 16))
    wait(fi_cp)
    _interleave(part(5, MS), (each(inv, range(3)), 96))
    fence()
    _interleave(part(6, MS), (finish(), 32 * N2 // QF))
    o_cp(0, S - MB).start()
    _interleave(mlp_stream([(r, MS, nf + n) for r in range(S - MB, S, MS) for n in range(nd)], MS))
    wait(o_cp(0, S - MB), *[o_cp(r, MS) for r in range(S - MB, S - MS, MS)], *end_cp)


@jax.jit
def pallas_recurrent_scan__spectral_gfnet__swiglu_ffn__prompt_kernel(
    A_x: jax.Array,
    A_w_r: jax.Array,
    A_w_i: jax.Array,
    B_x: jax.Array,
    B_w_gate: jax.Array,
    B_w_up: jax.Array,
    B_w_down: jax.Array,
):
    del B_x
    consts = _constants()
    vm = pltpu.VMEM
    pk = lambda *sh: vm((*sh[:-2], sh[-2] // 2, sh[-1]), jnp.uint32)
    scratch = [
        vm((S, D), BF), vm((DF, S), BF), vm((DF, S), BF), vm((D, F), BF), vm((D, F), BF), vm((F, D), BF),
        *[vm(c.shape, c.dtype) for c in consts],
        pk(S, D),
        pk(S, D),
        vm((3, 2, S, L), F32),
        vm((3, 2, S, L), F32),
        vm((3, N1, 2 * N2, L), F32),
        pk(2, 2, DF + 15, L),
        vm((3, WP * N2 + N1, L), jnp.uint32),
        vm((S, D), F32),
        pk(2 * MB, F),
        pk(5, KH, F),
        pk(5, (S - MB) // 2, KH),
        pk(5, F // 2, FC),
        pk(2, 5, SH, F // 2),
        vm((2, 2, SH, FC), F32),
        vm((S, D), BF),
        pltpu.SemaphoreType.DMA((S // RB,)),
        pltpu.SemaphoreType.DMA((2 * F // FC + 2,)),
        pltpu.SemaphoreType.DMA((7,)),
        pltpu.SemaphoreType.DMA((S // MS,)),
        pltpu.SemaphoreType.REGULAR,
    ]
    out = pl.pallas_call(
        _kernel,
        out_shape=jax.ShapeDtypeStruct((S, D), BF),
        in_specs=[pl.BlockSpec(memory_space=pltpu.HBM)] * 10,
        out_specs=pl.BlockSpec(memory_space=pltpu.HBM),
        scratch_shapes=scratch,
        compiler_params=pltpu.CompilerParams(
            vmem_limit_bytes=100 * 1024 * 1024, flags={"XLA_TPU_EVENLY_DISTRIBUTE_CRITICAL_NODES": True}),
    )(A_x.reshape(S, D), A_w_r.T, A_w_i.T, B_w_gate, B_w_up, B_w_down, *consts)
    return out.reshape(A_x.shape)
```
